```python
import os as _os
_os.environ.setdefault("JAX_PLATFORMS", "cpu")
import jax
import jax.numpy as jnp

def _softmax(x, axis=-1):
    return jax.nn.softmax(x, axis=axis)
def _gelu(x):
    return jax.nn.gelu(x, approximate=True)
def _silu(x):
    return jax.nn.silu(x)
def _sigmoid(x):
    return jax.nn.sigmoid(x)
def _layernorm(x, axis=-1, eps=1e-5):
    m = jnp.mean(x, axis=axis, keepdims=True)
    v = jnp.var(x, axis=axis, keepdims=True)
    return (x - m) / jnp.sqrt(v + eps)
def _scatter_add(tgt, idx, src, axis=0):
    return tgt.at[idx].add(src)
def _segment_sum(src, seg, n):
    return jax.ops.segment_sum(src, seg, n)
class _Rng:
    def __init__(self, key):
        self._k = key
    def _next(self):
        self._k, sub = jax.random.split(self._k)
        return sub
    def normal(self, shape):
        return jax.random.normal(self._next(), shape, dtype=jnp.bfloat16)
    def randint(self, lo, hi, shape):
        return jax.random.randint(self._next(), shape, lo, hi, dtype=jnp.int32)
    def uniform(self, shape, lo=0.0, hi=1.0):
        return jax.random.uniform(self._next(), shape, jnp.bfloat16, lo, hi)
    def permutation(self, n):
        return jax.random.permutation(self._next(), n)


kernel_name = 'concat_heads__gqa_block_cached__sliding_block_cached__decode'

def setup_inputs():
    _rng = _Rng(jax.random.key(int.from_bytes(__import__("os").urandom(4), "little")))
    _w = (lambda a: (lambda t: t.astype(jnp.bfloat16) if jnp.issubdtype(t.dtype, jnp.floating) else t)(jnp.asarray(a)))
    def _A_setup():
        B, Sq, D = 1, 1, 576
        Hq, Hkv, Sk, Dh = 32, 16, 8192, 128
        assert Hq % Hkv == 0, (Hq, Hkv)
        return {
            "x": _w((lambda *s: _rng.normal(s) * 0.8)(B, Sq, D)),
            "k_cache": _w((lambda *s: _rng.normal(s) * 0.8)(B, Hkv, Sk, Dh)),
            "v_cache": _w((lambda *s: _rng.normal(s) * 0.05)(B, Hkv, Sk, Dh)),
            "wq": _w((lambda *s: _rng.normal(s) * 0.8)(D, Hq * Dh) * (D ** -0.5)),
            "wo": _w((lambda *s: _rng.normal(s) * 0.05)(Hq * Dh, D) * ((Hq * Dh) ** -0.5)),
        }
    _A_in = _A_setup()

    def _B_setup():
        B, Sq, D = 1, 1, 576
        Hq, Hkv, Sk, Dh = 32, 16, 8192, 128
        assert Hq % Hkv == 0, (Hq, Hkv)
        return {
            "x": _w((lambda *s: _rng.normal(s) * 0.8)(B, Sq, D)),
            "k_cache": _w((lambda *s: _rng.normal(s) * 0.8)(B, Hkv, Sk, Dh)),
            "v_cache": _w((lambda *s: _rng.normal(s) * 0.05)(B, Hkv, Sk, Dh)),
            "wq": _w((lambda *s: _rng.normal(s) * 0.8)(D, Hq * Dh) * (D ** -0.5)),
            "wo": _w((lambda *s: _rng.normal(s) * 0.05)(Hq * Dh, D) * ((Hq * Dh) ** -0.5)),
        }
    _B_in = _B_setup()

    return {
        "A_x": _A_in["x"],
        "A_k_cache": _A_in["k_cache"],
        "A_v_cache": _A_in["v_cache"],
        "A_wq": _A_in["wq"],
        "A_wo": _A_in["wo"],
        "B_x": _B_in["x"],
        "B_k_cache": _B_in["k_cache"],
        "B_v_cache": _B_in["v_cache"],
        "B_wq": _B_in["wq"],
        "B_wo": _B_in["wo"],
    }

def reference(A_x, A_k_cache, A_v_cache, A_wq, A_wo, B_x, B_k_cache, B_v_cache, B_wq, B_wo):
    def _A_ref(x, k_cache, v_cache, wq, wo):
        B, Sq, D = x.shape
        Hq, Dh = 32, 128
        Hkv = k_cache.shape[1]
        rep = Hq // Hkv
        q = (lambda x, *d: x.transpose(*d))((x @ wq).reshape(B, Sq, Hq, Dh), 0, 2, 1, 3)
        k = jnp.repeat(k_cache, rep, axis=1)
        v = jnp.repeat(v_cache, rep, axis=1)
        scores = jnp.einsum("bhqd,bhkd->bhqk", q, k) * (Dh ** -0.5)
        p = _softmax(scores, axis=-1)
        o = jnp.einsum("bhqk,bhkd->bhqd", p, v)
        return (lambda x, *d: x.transpose(*d))(o, 0, 2, 1, 3).reshape(B, Sq, Hq * Dh) @ wo

    def _B_ref(x, k_cache, v_cache, wq, wo):
        B, Sq, D = x.shape
        Hq, Dh = 32, 128
        Hkv, Sk = k_cache.shape[1], k_cache.shape[2]
        W = min(4096, max(256, Sk // 4))
        rep = Hq // Hkv
        q = (lambda x, *d: x.transpose(*d))((x @ wq).reshape(B, Sq, Hq, Dh), 0, 2, 1, 3)
        k = jnp.repeat(k_cache[:, :, Sk - W:, :], rep, axis=1)
        v = jnp.repeat(v_cache[:, :, Sk - W:, :], rep, axis=1)
        scores = jnp.einsum("bhqd,bhkd->bhqk", q, k) * (Dh ** -0.5)
        p = _softmax(scores, axis=-1)
        o = jnp.einsum("bhqk,bhkd->bhqd", p, v)
        return (lambda x, *d: x.transpose(*d))(o, 0, 2, 1, 3).reshape(B, Sq, Hq * Dh) @ wo

    a = _A_ref(A_x, A_k_cache, A_v_cache, A_wq, A_wo)
    b = _B_ref(B_x, B_k_cache, B_v_cache, B_wq, B_wo)
    return jnp.concatenate([a, b], axis=-1)
```

```python
import functools
import jax, jax.numpy as jnp
from jax import lax
import jax.experimental.pallas as pl
import jax.experimental.pallas.tpu as pltpu

bf, f32 = jnp.bfloat16, jnp.float32
NT = (((1,), (1,)), ((), ()))
SCALE = 128 ** -0.5

def make(compute_only=False):
    def kern(ax, ak, av, awq, awo, bx, bk, bv, bwq, bwo, o_ref, xbuf, wbuf, kbuf, vbuf, q_scr, o_scr, xsem, wsem, ksem, vsem):
        row = lax.broadcasted_iota(jnp.int32, (8, 128), 0)
        wq_cp = [pltpu.make_async_copy(w, wbuf.at[i], wsem.at[i]) for i, w in enumerate((awq, bwq))]
        wo_cp = [pltpu.make_async_copy(w, wbuf.at[2 + i], wsem.at[2 + i]) for i, w in enumerate((awo, bwo))]
        x_cp = [pltpu.make_async_copy(x.at[0], xbuf.at[i], xsem.at[i]) for i, x in enumerate((ax, bx))]
        def kv_cp(src, buf, sem, h, n):
            slot = h % 2
            return pltpu.make_async_copy(src.at[0, h, pl.ds(8192 - n, n), :], buf.at[slot, pl.ds(0, n), :], sem.at[slot])
        def start(c):
            if not compute_only: c.start()
            else: c._used = True
        def wait(c):
            if not compute_only: c.wait()
            else: c._used = True
        start(wq_cp[0]); start(x_cp[0]); start(x_cp[1]); start(wq_cp[1])
        start(kv_cp(ak, kbuf, ksem, 0, 8192)); start(kv_cp(av, vbuf, vsem, 0, 8192))
        for i in range(2):
            wait(x_cp[i]); wait(wq_cp[i])
            x8 = jnp.broadcast_to(xbuf[i], (8, 576))
            for g in range(4):
                r = jnp.dot(x8, wbuf[i, :, g*1024:(g+1)*1024], preferred_element_type=f32)
                q = r[:, 0:128]
                for j in range(1, 8):
                    q = jnp.where(row == j, r[:, j*128:(j+1)*128], q)
                q_scr[i*4 + g] = q
        def head(h, i, ksrc, vsrc, n, nxt):
            slot = h % 2
            nxt()
            wait(kv_cp(ksrc, kbuf, ksem, h, n))
            q = q_scr[i*4 + h // 4].astype(bf)
            s = lax.dot_general(q, kbuf[slot, 0:n, :], NT, preferred_element_type=f32) * SCALE
            m = jnp.max(s, axis=1, keepdims=True)
            p = jnp.exp(s - m)
            l = jnp.sum(p, axis=1, keepdims=True)
            wait(kv_cp(vsrc, vbuf, vsem, h, n))
            acc = jnp.dot(p.astype(bf), vbuf[slot, 0:n, :], preferred_element_type=f32) / l
            for r in range(2):
                o_scr[i, 2*h + r] = jnp.where(row == (2*h + r) % 8, acc, 0.0)
        def bodyA(h, _):
            def nxt():
                @pl.when(h < 15)
                def _():
                    start(kv_cp(ak, kbuf, ksem, h + 1, 8192)); start(kv_cp(av, vbuf, vsem, h + 1, 8192))
                @pl.when(h == 15)
                def _():
                    start(kv_cp(bk, kbuf, ksem, 0, 2048)); start(kv_cp(bv, vbuf, vsem, 0, 2048))
                    start(wo_cp[0])
            head(h, 0, ak, av, 8192, nxt)
        lax.fori_loop(0, 16, bodyA, None)
        def oproj(i):
            wait(wo_cp[i])
            lhs = jnp.concatenate([o_scr[i, n] for n in range(32)], axis=1).astype(bf)
            r = lax.dot_general(lhs, wbuf[2 + i], NT, preferred_element_type=f32)
            return jnp.sum(r, axis=0, keepdims=True)
        def bodyB(h, _):
            def nxt():
                @pl.when(h < 15)
                def _():
                    start(kv_cp(bk, kbuf, ksem, h + 1, 2048)); start(kv_cp(bv, vbuf, vsem, h + 1, 2048))
                @pl.when(h == 15)
                def _():
                    start(wo_cp[1])
            head(h, 1, bk, bv, 2048, nxt)
        lax.fori_loop(0, 16, bodyB, None)
        oa = oproj(0)
        ob = oproj(1)
        o_ref[0] = jnp.concatenate([oa, ob], axis=1).astype(bf)

    def f(A_x,A_k,A_v,A_wq,A_wo,B_x,B_k,B_v,B_wq,B_wo):
        return pl.pallas_call(kern, in_specs=[pl.BlockSpec(memory_space=pltpu.HBM)]*10,
            out_shape=jax.ShapeDtypeStruct((1,1,1152),bf),
            scratch_shapes=[pltpu.VMEM((2,1,576), bf), pltpu.VMEM((4,576,4096), bf), pltpu.VMEM((2,8192,128), bf), pltpu.VMEM((2,8192,128), bf),
                            pltpu.VMEM((8,8,128), f32), pltpu.VMEM((2,32,8,128), f32),
                            pltpu.SemaphoreType.DMA((2,)), pltpu.SemaphoreType.DMA((4,)), pltpu.SemaphoreType.DMA((2,)), pltpu.SemaphoreType.DMA((2,))],
            compiler_params=pltpu.CompilerParams(vmem_limit_bytes=100*2**20, disable_bounds_checks=True),
            name="v1",
            )(A_x,A_k,A_v,A_wq,A_wo.T,B_x,B_k,B_v,B_wq,B_wo.T)
    return f


@jax.jit
def pallas_concat_heads__gqa_block_cached__sliding_block_cached__decode_kernel(
    A_x, A_k_cache, A_v_cache, A_wq, A_wo, B_x, B_k_cache, B_v_cache, B_wq, B_wo):
    return make()(A_x, A_k_cache, A_v_cache, A_wq, A_wo, B_x, B_k_cache, B_v_cache, B_wq, B_wo)
```

```python
import functools
import jax, jax.numpy as jnp
from jax import lax
import jax.experimental.pallas as pl
import jax.experimental.pallas.tpu as pltpu

bf, f32 = jnp.bfloat16, jnp.float32
NT = (((1,), (1,)), ((), ()))
SCALE = 128 ** -0.5
HI, LO = 0, 1

def make(D=4, R=8, d_wq=72, d_wo=(1, 60, 60), d_kv=(1, 70, 70), pin=True, name="v3", flags=None, nosem=False):
    NA, NB = 256, 64
    assert R >= D + 3 and R & (R - 1) == 0
    def kern(ax, ak, av, awq, awo, bx, bk, bv, bwq, bwo, o_ref,
             xbuf, wq, wo, kbuf, vbuf, q_scr, o_scr, y_scr, xsem, qsem, lsem, hsem):
        row = lax.broadcasted_iota(jnp.int32, (8, 128), 0)
        lane = lax.broadcasted_iota(jnp.int32, (8, 128), 1)
        def delay(ns):
            if ns: pl.delay(ns)
        def ds(start, size, align=None):
            return pl.ds(start if isinstance(start, int) else pl.multiple_of(start, align or size), size)
        def wq_cp(i, k, b):
            rows = ds(64*b + 8*(k >> 1), 8)
            cols = ds((k & 1) * 2048, 2048)
            return pltpu.make_async_copy((awq, bwq)[i].at[rows, cols], wq.at[i, rows, cols], qsem.at[i, k & 1])
        def wq_wait(k):
            for i in range(2):
                d = wq.at[i, pl.ds(0, 72), pl.ds(0, 2048)]
                pltpu.make_async_copy(d, d, qsem.at[i, k & 1]).wait()
        def slot_wait(t):
            s = t & (R - 1)
            pltpu.make_async_copy(kbuf.at[s], kbuf.at[s], lsem.at[s]).wait()
            pltpu.make_async_copy(vbuf.at[s], vbuf.at[s], hsem.at[s]).wait()
        def wo_issue(t, u):
            r = 64*((t & 1) * 4 + u) + 8*(t >> 2)
            cols = ds(((t >> 1) & 1) * 2048, 2048)
            s = t & (R - 1)
            pltpu.make_async_copy(bwo.at[ds(r + 64, 8), cols], wo.at[ds(r + 640, 8), cols], hsem.at[s]).start(priority=HI)
            pltpu.make_async_copy(awo.at[ds(r, 8), cols], wo.at[ds(r, 8), cols], lsem.at[s]).start(priority=LO)
        def kv_issue(ksrc, vsrc, lg):
            def issue(t, u):
                g = t >> lg; c = t & ((1 << lg) - 1)
                rows = ds(8192 - (128 << lg) + c*128, 128)
                s = t & (R - 1)
                pltpu.make_async_copy(vsrc.at[0, 4*g + u, rows], vbuf.at[s, pl.ds(128*u, 128)], hsem.at[s]).start(priority=HI)
                pltpu.make_async_copy(ksrc.at[0, 4*g + u, rows], kbuf.at[s, pl.ds(128*u, 128)], lsem.at[s]).start(priority=LO)
            return issue
        a_issue = kv_issue(ak, av, 6); b_issue = kv_issue(bk, bv, 4)
        def mid_issue(t, u):
            cols = ds(t * 1024, 1024)
            s = t & (R - 1)
            pltpu.make_async_copy(bwo.at[pl.ds(16*u, 16), cols], wo.at[pl.ds(576 + 16*u, 16), cols], hsem.at[s]).start(priority=HI)
            pltpu.make_async_copy(awo.at[pl.ds(512 + 16*u, 16), cols], wo.at[pl.ds(512 + 16*u, 16), cols], lsem.at[s]).start(priority=LO)

        x_cp = [pltpu.make_async_copy(x.at[0], xbuf.at[i], xsem.at[i]) for i, x in enumerate((ax, bx))]
        for b in range(9): wq_cp(0, 0, b).start(priority=LO)
        def wq_head(b, _):
            wq_cp(1, 0, b).start(priority=HI)
            wq_cp(0, 1, b).start(priority=LO)
            delay(d_wq)
        lax.fori_loop(0, 9, wq_head, None)
        x_cp[0].start(); x_cp[1].start()
        def wq_head2(b, _):
            wq_cp(1, 1, b).start(priority=HI)
            delay(d_wq)
        lax.fori_loop(0, 5, wq_head2, None)
        for b in range(5, 9): wq_cp(1, 1, b).start(priority=LO)
        delay(4*d_wq)
        def wq_body(k, _):
            wq_wait(k)
            def inner(b, _):
                wq_cp(1, k + 2, b).start(priority=HI)
                wq_cp(0, k + 2, b).start(priority=LO)
                delay(d_wq)
            lax.fori_loop(0, 9, inner, None)
        lax.fori_loop(0, 14, wq_body, None)
        def trans(lo_, hi_):
            def inner(n, _):
                wo_issue(n >> 2, n & 3)
                delay(d_wq)
            lax.fori_loop(lo_, hi_, inner, None)
        wq_wait(14); trans(0, 2*D); wq_wait(15); trans(2*D, 4*D)
        x_cp[0].wait(); x_cp[1].wait()
        x8 = [jnp.broadcast_to(xbuf[i], (8, 576)) for i in range(2)]

        def q_body(issue, off):
            def body(t, qs):
                slot_wait(t)
                issue(t + D - off, 0)
                delay(1)
                cols = ds(t * 128, 128)
                out = []
                for i in range(2):
                    r = jnp.dot(x8[i], wq[i, :, cols], preferred_element_type=f32)
                    q = jnp.where(row == (t & 7), r, qs[i])
                    q_scr[4*i + (t >> 3)] = q
                    out.append(q)
                for u in range(1, 4):
                    issue(t + D - off, u); delay(d_wo[u-1])
                return tuple(out)
            return body
        z = jnp.zeros((8, 128), f32)
        qs = lax.fori_loop(0, 32 - D, q_body(wo_issue, 0), (z, z))
        lax.fori_loop(32 - D, 32, q_body(a_issue, 32), qs)
        y_scr[...] = jnp.zeros(y_scr.shape, f32)

        def oproj(gg, j):
            i = gg >> 2
            cols = ds(((gg & 3) * 8 + j) * 128, 128)
            r = lax.dot_general(o_scr[gg].astype(bf), wo[ds(i * 640, 512, 128), cols], NT, preferred_element_type=f32)
            y_scr[i] += jnp.where(lax.broadcasted_iota(jnp.int32, (8, 512), 0) == j, r, 0.0)
        def pos(t):
            isA = t < NA
            return jnp.where(isA, t >> 6, (t >> 4) - (NA // 16 - 4)), jnp.where(isA, t & 63, t & 15)
        def qk(t):
            gg, _ = pos(t)
            r = lax.dot_general(q_scr[gg].astype(bf), kbuf[t & (R - 1)], NT, preferred_element_type=f32)
            s = r[:, 0:128]
            for u in range(1, 4):
                s = jnp.where(row >= 2*u, r[:, 128*u:128*(u+1)], s)
            return s * SCALE
        def sm(t, s, m):
            _, c = pos(t)
            m_old = jnp.where(c == 0, -jnp.inf, m)
            m_new = jnp.maximum(m_old, jnp.max(s, axis=1, keepdims=True))
            return m_new, jnp.exp(s - m_new), jnp.exp(m_old - m_new)
        def pv(t, p, alpha, l, acc):
            _, c = pos(t)
            s_ = jnp.maximum(t, 0) & (R - 1)
            pb = p.astype(bf)
            r = jnp.dot(pb, vbuf[s_, 0:128], preferred_element_type=f32)
            for u in range(1, 4):
                r = jnp.where(row >= 2*u, jnp.dot(pb, vbuf[s_, 128*u:128*(u+1)], preferred_element_type=f32), r)
            first = c == 0
            return jnp.where(first, 0.0, l * alpha) + p, jnp.where(first, 0.0, acc * alpha) + r
        def kv_body(issue, off):
            def body(t, carry):
                s, m, p, alpha, l, acc = carry
                slot_wait(t)
                issue(t + D - off, 0)
                delay(1)
                l, acc = pv(t - 2, p, alpha, l, acc)
                s_new = qk(t)
                m, p, alpha = sm(t - 1, s, m)
                if pin:
                    vbuf[R + (t & 1), 0:8] = p.astype(bf)
                issue(t + D - off, 1)
                delay(d_kv[0])
                issue(t + D - off, 2)
                gg, c = pos(t)
                fin = jnp.logical_and(gg > 0, c == 1)
                @pl.when(fin)
                def _():
                    o_scr[gg - 1] = acc / jnp.sum(l, axis=1, keepdims=True)
                do_op = jnp.logical_and(gg > 0, jnp.logical_and(c >= 2, c < 10))
                @pl.when(do_op)
                def _():
                    oproj(gg - 1, c - 2)
                @pl.when(jnp.logical_not(jnp.logical_or(fin, do_op)))
                def _():
                    delay(d_kv[1])
                issue(t + D - off, 3)
                @pl.when(jnp.logical_not(do_op))
                def _():
                    delay(d_kv[2])
                return s_new, m, p, alpha, l, acc
            return body
        cy = lax.fori_loop(0, NA - D, kv_body(a_issue, 0), (y_scr[0, :, 0:128],)*6)
        cy = lax.fori_loop(NA - D, NA + NB - D, kv_body(b_issue, NA), cy)
        assert D >= 4
        cy = lax.fori_loop(NA + NB - D, NA + NB - D + 4, kv_body(mid_issue, NA + NB), cy)
        if D > 4:
            cy = lax.fori_loop(NA + NB - D + 4, NA + NB, kv_body(lambda t, u: None, 0), cy)
        s, m, p, alpha, l, acc = cy
        T = NA + NB
        l, acc = pv(T - 2, p, alpha, l, acc)
        m, p, alpha = sm(T - 1, s, m)
        l, acc = pv(T - 1, p, alpha, l, acc)
        o_scr[7] = acc / jnp.sum(l, axis=1, keepdims=True)
        def op2(j, _):
            for jj in range(4): oproj(7, 4*j + jj)
        lax.fori_loop(0, 2, op2, None)
        ya = jnp.sum(y_scr[0], axis=0, keepdims=True); yb = jnp.sum(y_scr[1], axis=0, keepdims=True)
        o_ref[0, :, 0:512] = ya.astype(bf)
        o_ref[0, :, 640:1152] = yb.astype(bf)
        def mid_body(g, y):
            lhs = jnp.concatenate([o_scr[g], o_scr[4 + g]], axis=0).astype(bf)
            slot_wait(g)
            for j in range(8):
                cols = ds((g * 8 + j) * 128, 128)
                r = lax.dot_general(lhs, wo[512:640, cols], NT, preferred_element_type=f32)
                y = y + jnp.where(row == j, jnp.where(lane < 64, r[0:8], r[8:16]), 0.0)
            return y
        y = lax.fori_loop(0, 4, mid_body, z)
        o_ref[0, :, 512:640] = jnp.sum(y, axis=0, keepdims=True).astype(bf)

    def f(A_x,A_k,A_v,A_wq,A_wo,B_x,B_k,B_v,B_wq,B_wo):
        return pl.pallas_call(kern, in_specs=[pl.BlockSpec(memory_space=pltpu.HBM)]*10,
            out_shape=jax.ShapeDtypeStruct((1,1,1152),bf),
            scratch_shapes=[pltpu.VMEM((2,1,576), bf), pltpu.VMEM((2,576,4096), bf), pltpu.VMEM((1152,4096), bf),
                            pltpu.VMEM((R,512,128), bf), pltpu.VMEM((R+2,512,128), bf),
                            pltpu.VMEM((8,8,128), f32), pltpu.VMEM((8,8,128), f32), pltpu.VMEM((2,8,512), f32),
                            pltpu.SemaphoreType.DMA((2,)), pltpu.SemaphoreType.DMA((2,2)), pltpu.SemaphoreType.DMA((R,)), pltpu.SemaphoreType.DMA((R,))],
            compiler_params=pltpu.CompilerParams(vmem_limit_bytes=64*2**20, disable_bounds_checks=True, disable_semaphore_checks=nosem, flags=flags),
            name=name,
            )(A_x,A_k,A_v,A_wq,A_wo.T,B_x,B_k,B_v,B_wq,B_wo.T)
    return f


@jax.jit
def pallas_concat_heads__gqa_block_cached__sliding_block_cached__decode_kernel(
    A_x, A_k_cache, A_v_cache, A_wq, A_wo, B_x, B_k_cache, B_v_cache, B_wq, B_wo):
    return make(d_kv=(1,60,60), d_wo=(1,40,40), nosem=True)(A_x, A_k_cache, A_v_cache, A_wq, A_wo, B_x, B_k_cache, B_v_cache, B_wq, B_wo)
```

```python
import functools
import jax, jax.numpy as jnp
from jax import lax
import jax.experimental.pallas as pl
import jax.experimental.pallas.tpu as pltpu

bf, f32 = jnp.bfloat16, jnp.float32
NT = (((1,), (1,)), ((), ()))
SCALE = 128 ** -0.5
HI, LO = 0, 1

def make(D=4, strided=True, aswap=False, bswap=False, kord=0, notail=0, blocks=((0,),(1,2),(3,)), finsplit=False, nseg=1, lmode=0, wm=2, w2=6, bwm=None, bsingle=False, R=8, d0=50, d_wq=72, d_wo=(1, 40, 40), d_kv=(1, 52, 52), d_last=(1, 1, 60, 60), pin=True, shift_b=True, rot_a=0, name="v7", flags=None, scopes=False):
    NW, NB, NA = 36, 64, 256
    T = NA + NB
    assert R >= D + 3 and R & (R - 1) == 0 and (2 * NW) % R == 0 and T % R == 0 and NB % R == 0
    import contextlib
    scope = jax.named_scope if scopes else (lambda n: contextlib.nullcontext())
    def kern(ax, ak, av, awq, awo, bx, bk, bv, bwq, bwo, o_ref,
             xbuf, wq, wo, kbuf, vbuf, q_scr, o_scr, y_scr, xsem, lsem, hsem):
        row = lax.broadcasted_iota(jnp.int32, (8, 128), 0)
        def delay(ns):
            if ns: pl.delay(ns)
        def ds(start, size, align=None):
            return pl.ds(start if isinstance(start, int) else pl.multiple_of(start, align or size), size)
        def copy(src, dst, sem, prio):
            pltpu.make_async_copy(src, dst, sem).start(priority=prio)
        def wait(sem, n, rows=512):
            d = kbuf.at[0, pl.ds(0, rows // 128)]
            pltpu.make_async_copy(d, d, sem.at[n & (R - 1)]).wait()
        def w_piece(src, dst, m, ncol, sem, prio):
            k = (m * 57) >> 9
            b = (m - 9 * k) * wm
            b = b - 9 * ((b * 57) >> 9)
            if kord == 0:
                r = k >> 2 if ncol == 4 else (k * 11) >> 5
                c = k - ncol * r
            else:
                r = k & 7; c = k >> 3
            rows, cols = ds(64 * b + 8 * r, 8), ds(1024 * c, 1024)
            copy(src.at[rows, cols], dst.at[rows, cols], sem, prio)
        def w_issue(a_src, b_src, a_dst, b_dst, ncol, first):
            def issue(n, u, hi=True, lo=True):
                s = n & (R - 1); n = n - first
                if hi:
                    for e in range(ncol * u // 2, ncol * (u + 1) // 2):
                        w_piece(a_src, a_dst, 2 * ncol * n + e, ncol, hsem.at[s], HI)
                if lo:
                    for e in range(2):
                        w_piece(b_src, b_dst, 8 * n + 2 * u + e, 4, lsem.at[s], LO)
            return issue
        wq_issue = w_issue(awq, bwq, wq.at[0], wq.at[1], 4, 0)
        wo_issue = w_issue(awo, bwo, wo.at[pl.ds(0, 576)], wo.at[pl.ds(576, 576)], 3, NW)
        def b_issue(n, u):
            s = n & (R - 1)
            j = 2 * (u & 1); e = u >> 1
            h = 4 * (n >> 4) + j; rows = ds(6144 + 128 * (n & 15) + 64 * e, 64)
            for src, buf, sem, prio in ((bk, kbuf, hsem, HI), (bv, vbuf, lsem, LO)):
                if bswap:
                    for i in range(2): copy(src.at[h - j + (u & 1) + 2*i, rows], buf.at[s, (u & 1) + 2*i, e], sem.at[s], prio)
                elif strided:
                    copy(src.at[pl.ds(h, 2), rows], buf.at[s, pl.ds(j, 2), e], sem.at[s], prio)
                else:
                    for i in range(2): copy(src.at[h + i, rows], buf.at[s, j + i, e], sem.at[s], prio)
        def a_issue(n, u):
            n = n - NB
            if aswap: u = (0, 2, 1, 3)[u]
            h = 4 * (n >> 6) + u; rows = ds(64 * (n & 63), 64); s = n & (R - 1)
            for src, buf, sem, prio in ((ak, kbuf, hsem, HI), (av, vbuf, lsem, LO)):
                if strided:
                    copy(src.at[h, :, rows], buf.at[s, u], sem.at[s], prio)
                else:
                    for e in range(2): copy(src.at[h, e, rows], buf.at[s, u, e], sem.at[s], prio)
        def last_copy(r0, r1, sem, prio):
            for r in (r0, r1):
                copy(awo.at[ds(r, 8), pl.ds(3072, 1024)], wo.at[ds(r, 8), pl.ds(3072, 1024)], sem, prio)
        def last_issue(n, u):
            j = n - T
            if lmode == 0:
                r = 128 * (j >> 1) + 32 * (j & 1) + 8 * u
                last_copy(r, r + 64, hsem.at[j], HI)
            else:
                r = 16 * j + 8 * (u >> 1) + 64 * (u & 1)
                last_copy(r, r + 128, hsem.at[j], HI)
                r = 128 * (j >> 1) + 32 * (j & 1) + 8 * u
            last_copy(256 + r, 320 + r, lsem.at[j], LO)

        x_cp = [pltpu.make_async_copy(x.at[0], xbuf.at[i], xsem) for i, x in enumerate((ax, bx))]
        for n in range(2):
            for u in range(4): wq_issue(n, u, hi=False)
        def head(n, _):
            for u in range(4):
                wq_issue(n, u, lo=False); delay(d0)
        with scope("p0"): lax.fori_loop(0, 2, head, None)
        x_cp[0].start(); x_cp[1].start()
        def stream(issue, hrows, d):
            def body(n, _):
                @pl.when(n >= D)
                def _(): wait(hsem, n - D, hrows)
                @pl.when(n >= D + 2)
                def _(): wait(lsem, n - D - 2)
                for u in range(4):
                    issue(n, u); delay(d)
            return body
        with scope("p1_wq"): lax.fori_loop(2, NW, stream(wq_issue, 512, d_wq), None)
        with scope("p1_tr"): lax.fori_loop(NW, NW + D, stream(wo_issue, 512, d_wq - 10), None)
        x_cp[0].wait(); x_cp[1].wait()
        x8 = [jnp.broadcast_to(xbuf[i], (8, 576)) for i in range(2)]
        y_scr[...] = jnp.zeros(y_scr.shape, f32)
        wo[512:576, 3072:4096] = jnp.zeros((64, 1024), bf)
        z = y_scr[0]
        wait(lsem, NW - 2)
        def q_body(t, qs):
            wait(hsem, NW + t, 384); wait(lsem, NW + t - 1)
            wo_issue(NW + t + D, 0)
            delay(1)
            cols = ds(t * 128, 128)
            out = []
            for i in range(2):
                r = jnp.dot(x8[i], wq[i, :, cols], preferred_element_type=f32)
                q = jnp.where(row == (t & 7), r, qs[i])
                q_scr[4*(1 - i) + (t >> 3)] = q
                out.append(q)
            for u in range(1, 4):
                wo_issue(NW + t + D, u); delay(d_wo[u-1])
            return tuple(out)
        with scope("p2_q"): lax.fori_loop(0, 32, q_body, (z, z))
        assert D in (3, 4)
        wait(hsem, NW + 32, 384)
        if D == 3:
            for u in range(4):
                wo_issue(2*NW - 1, u); delay(d_wq - 10)
        else:
            for u in range(4):
                b_issue(0, u); delay(d_wq)
        def pre(t, _):
            wait(hsem, t, 384); wait(lsem, t - 2)
            def inner(u, _):
                b_issue(t + D - 2*NW, u); delay(d_wq)
            lax.fori_loop(0, 4, inner, None)
        with scope("p2_tr"): lax.fori_loop(NW + 33, 2*NW, pre, None)

        def oproj(gg, j):
            i = 1 - (gg >> 2)
            cols = ds(((gg & 3) * 2 + (j & 1)) * 512, 512)
            y_scr[5 * i + (j >> 1)] += lax.dot_general(o_scr[j & 1], wo[ds(i * 512 + (j >> 1) * 128, 128), cols], NT, preferred_element_type=f32)
        def spread(o):
            return [jnp.concatenate([jnp.broadcast_to(o[j:j+1], (8, 128)) for j in range(4*e, 4*e + 4)], axis=1).astype(bf) for e in range(2)]
        def pos(t):
            isB = t < NB
            return jnp.where(isB, t >> 4, (t >> 6) + 3), jnp.where(isB, t & 15, t & 63)
        def qk(t):
            gg, _ = pos(t)
            r = lax.dot_general(q_scr[gg].astype(bf), kbuf[t & (R - 1)].reshape(512, 128), NT, preferred_element_type=f32)
            s = r[:, 0:128]
            for u in range(1, 4):
                s = jnp.where(row >= 2*u, r[:, 128*u:128*(u+1)], s)
            return s * SCALE
        def sm(t, s, m):
            _, c = pos(t)
            m_old = jnp.where(c == 0, -jnp.inf, m)
            m_new = jnp.maximum(m_old, jnp.max(s, axis=1, keepdims=True))
            return m_new, jnp.exp(s - m_new), jnp.exp(m_old - m_new)
        def pv(t, p, alpha, l, acc):
            _, c = pos(t)
            s_ = t & (R - 1)
            pb = p.astype(bf)
            r = jnp.dot(pb, vbuf[s_, 0].reshape(128, 128), preferred_element_type=f32)
            for u in range(1, 4):
                r = jnp.where(row >= 2*u, jnp.dot(pb, vbuf[s_, u].reshape(128, 128), preferred_element_type=f32), r)
            first = c == 0
            return jnp.where(first, 0.0, l * alpha) + p, jnp.where(first, 0.0, acc * alpha) + r
        def kv_body(issue, extras=True):
            def body(t, carry):
                s, m, p, alpha, l, acc = carry
                wait(hsem, t); wait(lsem, t - 2)
                issue(t + D, 0)
                delay(1)
                l, acc = pv(t - 2, p, alpha, l, acc)
                s_new = qk(t)
                m, p, alpha = sm(t - 1, s, m)
                if pin:
                    kbuf[R + (t & 1), 0, 0, 0:8] = p.astype(bf)
                issue(t + D, 1)
                delay(d_kv[0])
                issue(t + D, 2)
                if extras:
                    gg, c = pos(t)
                    fin = jnp.logical_and(gg > 0, c == 1)
                    @pl.when(fin)
                    def _():
                        o_scr[0], o_scr[1] = spread(acc / jnp.sum(l, axis=1, keepdims=True))
                    do_op = jnp.logical_and(gg > 0, jnp.logical_and(c >= 2, c < 12))
                    @pl.when(do_op)
                    def _():
                        oproj(gg - 1, c - 2)
                        issue(t + D, 3)
                    @pl.when(jnp.logical_not(do_op))
                    def _():
                        @pl.when(jnp.logical_not(fin))
                        def _():
                            delay(d_kv[1])
                        issue(t + D, 3)
                        delay(d_kv[2])
                else:
                    delay(d_kv[1]); issue(t + D, 3); delay(d_kv[2])
                return s_new, m, p, alpha, l, acc
            return body
        for s_ in (R - 2, R - 1):
            vbuf[s_] = jnp.zeros((4, 2, 64, 128), bf)
        with scope("p3_B"): cy = lax.fori_loop(0, NB - D, kv_body(b_issue), (z,)*6)
        for sg in range(nseg):
            with scope("p4_A"): cy = lax.fori_loop(NB - D + sg * NA // nseg, NB - D + (sg + 1) * NA // nseg, kv_body(a_issue), cy)
        for j in range(5):
            o_ref[0, :, 512 + 128*j:640 + 128*j] = y_scr[5 + j, 0:1].astype(bf)
        assert D == 4
        with scope("p4_l"): s, m, p, alpha, l, acc = lax.fori_loop(T - D, T, kv_body(last_issue, False), cy)
        fin_cp = pltpu.make_async_copy(awo.at[pl.ds(512, 64), pl.ds(3072, 1024)], wo.at[pl.ds(512, 64), pl.ds(3072, 1024)], lsem.at[4])
        if finsplit:
            for a in (0, 4, 1, 5, 2, 6, 3, 7):
                copy(awo.at[pl.ds(512 + 8*a, 8), pl.ds(3072, 1024)], wo.at[pl.ds(512 + 8*a, 8), pl.ds(3072, 1024)], lsem.at[4], LO)
        else:
            fin_cp.start(priority=LO)
        with scope("p5_0"):
            wait(lsem, T - 2)
            l, acc = pv(T - 2, p, alpha, l, acc)
            m, p, alpha = sm(T - 1, s, m)
        with scope("p5_1"):
            wait(lsem, T - 1)
            l, acc = pv(T - 1, p, alpha, l, acc)
            lhs = jnp.concatenate(spread(acc / jnp.sum(l, axis=1, keepdims=True)), axis=1)
        for blk in blocks:
            with scope("p5_w"):
                for j in blk:
                    for e in range(2): wait((hsem, lsem)[j >> 1], 2 * (j & 1) + e)
            for j in blk:
                if notail: continue
                r = lax.dot_general(lhs, wo[128*j:128*(j+1), 3072:4096], NT, preferred_element_type=f32)
                o_ref[0, :, 128*j:128*(j+1)] = (r[0:1] + y_scr[j, 0:1]).astype(bf)
        with scope("p5_w2"):
            fin_cp.wait()
        if notail == 2: return
        r = lax.dot_general(lhs, wo[512:576, 3072:4096], NT, preferred_element_type=f32)
        o_ref[0, :, 512:576] = (r[0:1] + y_scr[4, 0:1, 0:64]).astype(bf)

    def f(A_x,A_k,A_v,A_wq,A_wo,B_x,B_k,B_v,B_wq,B_wo):
        return pl.pallas_call(kern, in_specs=[pl.BlockSpec(memory_space=pltpu.HBM)]*10,
            out_shape=jax.ShapeDtypeStruct((1,1,1152),bf),
            scratch_shapes=[pltpu.VMEM((2,1,576), bf), pltpu.VMEM((2,576,4096), bf), pltpu.VMEM((1152,4096), bf),
                            pltpu.VMEM((R+2,4,2,64,128), bf), pltpu.VMEM((R,4,2,64,128), bf),
                            pltpu.VMEM((8,8,128), f32), pltpu.VMEM((2,8,512), bf), pltpu.VMEM((10,8,128), f32),
                            pltpu.SemaphoreType.DMA(()), pltpu.SemaphoreType.DMA((R,)), pltpu.SemaphoreType.DMA((R,))],
            compiler_params=pltpu.CompilerParams(vmem_limit_bytes=64*2**20, disable_bounds_checks=True, disable_semaphore_checks=True, flags=flags),
            name=name,
            )(A_x,A_k.reshape(16,2,4096,128),A_v.reshape(16,2,4096,128),A_wq,A_wo.T,B_x,B_k.reshape(16,8192,128),B_v.reshape(16,8192,128),B_wq,B_wo.T)
    return f


@jax.jit
def pallas_concat_heads__gqa_block_cached__sliding_block_cached__decode_kernel(
    A_x, A_k_cache, A_v_cache, A_wq, A_wo, B_x, B_k_cache, B_v_cache, B_wq, B_wo):
    return make()(A_x, A_k_cache, A_v_cache, A_wq, A_wo, B_x, B_k_cache, B_v_cache, B_wq, B_wo)
```

```python
import jax
import jax.numpy as jnp
from jax import lax
import jax.experimental.pallas as pl
import jax.experimental.pallas.tpu as pltpu

BF16, F32 = jnp.bfloat16, jnp.float32

D_MODEL, HQ, HKV, SK, DH = 576, 32, 16, 8192, 128
WINDOW = min(4096, max(256, SK // 4))
HID = HQ * DH

HI, LO = 0, 1
AHEAD = 4
RING = 8
NW = 36
NB = (HKV // 4) * (WINDOW // 128)
NA = (HKV // 4) * (SK // 128)
NT = NB + NA
LAST = HID - 8 * DH


def _ds(start, size):
    return pl.ds(start if isinstance(start, int) else pl.multiple_of(start, size), size)


def _div(m, d):
    return m // d


def _short_div(m, d):
    return (m * -(-512 // d)) >> 9


def _start(hi, lo):
    for copy in hi:
        copy.start(priority=HI)
    for copy in lo:
        copy.start(priority=LO)


def _wait(*groups):
    for group in groups:
        for copy in group:
            copy.wait()


def _dot_nt(a, b):
    return lax.dot_general(a, b, (((1,), (1,)), ((), ())), preferred_element_type=F32)


def _kernel(ax, ak, av, awq, awo, bx, bk, bv, bwq, bwo, o_ref,
            xbuf, wq, wo, kbuf, vbuf, q_scr, o_scr, y_scr, xsem, hsem, lsem):
    make_copy = pltpu.make_async_copy
    row = lax.broadcasted_iota(jnp.int32, (8, DH), 0)

    def no_stream(n, u):
        return []

    def weight_stream(src, dst, sem, ncol, first_step, div):
        def piece(m, s):
            k = div(m, 9)
            blk = 2 * (m - 9 * k)
            blk = blk - 9 * div(blk, 9)
            r = div(k, ncol)
            rows, cols = _ds(64 * blk + 8 * r, 8), _ds(1024 * (k - ncol * r), 1024)
            return make_copy(src.at[rows, cols], dst.at[rows, cols], sem.at[s])

        def stream(n, u):
            return [piece(2 * ncol * (n - first_step) + e, n & (RING - 1))
                    for e in range(ncol * u // 2, ncol * (u + 1) // 2)]
        return stream

    def b_stream(src, buf, sem):
        def stream(n, u):
            s, j, e = n & (RING - 1), 2 * (u & 1), u >> 1
            rows = _ds(SK - WINDOW + 128 * (n & 15) + 64 * e, 64)
            return [make_copy(src.at[pl.ds(4 * (n >> 4) + j, 2), rows],
                              buf.at[s, pl.ds(j, 2), e], sem.at[s])]
        return stream

    def a_stream(src, buf, sem):
        def stream(n, u):
            s = n & (RING - 1)
            return [make_copy(src.at[4 * ((n - NB) >> 6) + u, :, _ds(64 * (n & 63), 64)],
                              buf.at[s, u], sem.at[s])]
        return stream

    def last_copy(r, nrows, sem):
        idx = (_ds(r, nrows), pl.ds(LAST, HID - LAST))
        return make_copy(awo.at[idx], wo.at[idx], sem)

    def last_stream(first_row, sem):
        def stream(n, u):
            j = n - NT
            r = first_row + 128 * (j >> 1) + 32 * (j & 1) + 8 * u
            return [last_copy(r + 64 * e, 8, sem.at[j]) for e in range(2)]
        return stream

    wq_hi = weight_stream(awq, wq.at[0], hsem, 4, 0, _div)
    wq_lo = weight_stream(bwq, wq.at[1], lsem, 4, 0, _div)
    wo_hi = weight_stream(awo, wo.at[pl.ds(0, D_MODEL)], hsem, 3, NW, _short_div)
    wo_lo = weight_stream(bwo, wo.at[pl.ds(D_MODEL, D_MODEL)], lsem, 4, NW, _short_div)
    bk_hi, bv_lo = b_stream(bk, kbuf, hsem), b_stream(bv, vbuf, lsem)
    ak_hi, av_lo = a_stream(ak, kbuf, hsem), a_stream(av, vbuf, lsem)
    last_hi, last_lo = last_stream(0, hsem), last_stream(256, lsem)


    def stream_only(t0, t1, hi, lo, done_hi, done_lo):
        def body(t, _):
            for u in range(4):
                _wait(done_hi(t, u), done_lo(t - 1, u))
                _start(hi(t + AHEAD, u), lo(t + AHEAD, u))
        lax.fori_loop(t0, t1, body, None)

    for n in range(2):
        for u in range(4):
            _start([], wq_lo(n, u))
    stream_only(-AHEAD, 2 - AHEAD, wq_hi, no_stream, no_stream, no_stream)
    x_copies = [make_copy(x.at[0], xbuf.at[i], xsem) for i, x in enumerate((ax, bx))]
    _start(x_copies, [])
    stream_only(2 - AHEAD, 0, wq_hi, wq_lo, no_stream, no_stream)
    y_scr[...] = jnp.zeros(y_scr.shape, F32)
    wo[512:D_MODEL, LAST:HID] = jnp.zeros((D_MODEL - 512, HID - LAST), BF16)
    vbuf[RING - 1] = jnp.zeros(vbuf.shape[1:], BF16)
    stream_only(0, 1, wq_hi, wq_lo, wq_hi, no_stream)
    stream_only(1, NW - AHEAD, wq_hi, wq_lo, wq_hi, wq_lo)
    stream_only(NW - AHEAD, NW, wo_hi, wo_lo, wq_hi, wq_lo)
    stream_only(NW, NW + 1, wo_hi, wo_lo, wo_hi, wq_lo)
    stream_only(NW + 1, 2 * NW - HQ, wo_hi, wo_lo, wo_hi, wo_lo)

    _wait(x_copies)
    x8 = [jnp.broadcast_to(xbuf[i], (8, D_MODEL)) for i in range(2)]
    zero = y_scr[0]

    def q_step(hi, lo, first_step):
        def body(h, qs):
            t = 2 * NW - HQ + h
            n = t + AHEAD - first_step
            _wait(wo_hi(t, 0), wo_lo(t - 1, 0), wo_hi(t, 1), wo_lo(t - 1, 1))
            _start(hi(n, 0), lo(n, 0))
            slot2 = hi(n, 2), lo(n, 2)
            new_qs = []
            for i in range(2):
                r = jnp.dot(x8[i], wq[i, :, _ds(h * DH, DH)], preferred_element_type=F32)
                new_qs.append(jnp.where(row == (h & 7), r, qs[i]))
                q_scr[4 * (1 - i) + (h >> 3)] = new_qs[i]
            _start(hi(n, 1), lo(n, 1))
            _wait(wo_hi(t, 2), wo_lo(t - 1, 2))
            _start(*slot2)
            _wait(wo_hi(t, 3), wo_lo(t - 1, 3))
            _start(hi(n, 3), lo(n, 3))
            return tuple(new_qs)
        return body

    qs = lax.fori_loop(0, HQ - AHEAD, q_step(wo_hi, wo_lo, 0), (zero, zero))
    lax.fori_loop(HQ - AHEAD, HQ, q_step(bk_hi, bv_lo, 2 * NW), qs)

    def position(t):
        in_b = t < NB
        return jnp.where(in_b, t >> 4, (t >> 6) + 3), jnp.where(in_b, t & 15, t & 63)

    def wait_ring(buf, sem, n):
        s = n & (RING - 1)
        make_copy(buf.at[s], buf.at[s], sem.at[s]).wait()

    def own_rows(parts):
        out = parts[0]
        for u in range(1, 4):
            out = jnp.where(row >= 2 * u, parts[u], out)
        return out

    def accumulate(t, p, alpha, l, acc):
        first = position(t)[1] == 0
        pv = own_rows([
            jnp.dot(p.astype(BF16), vbuf[t & (RING - 1), u].reshape(128, DH),
                    preferred_element_type=F32) for u in range(4)])
        return jnp.where(first, 0.0, l * alpha) + p, jnp.where(first, 0.0, acc * alpha) + pv

    def normalize(l, acc):
        o = acc / jnp.sum(l, axis=1, keepdims=True)
        heads = [jnp.broadcast_to(o[j:j + 1], (8, DH)) for j in range(8)]
        return [jnp.concatenate(heads[4 * e:4 * e + 4], axis=1).astype(BF16) for e in range(2)]

    def attn_step(hi, lo, first=False):
        def body(t, carry):
            m, p, alpha, l, acc = carry
            g, c = position(t)
            n = t + AHEAD
            wait_ring(kbuf, hsem, t)
            if first:
                _wait(*[wo_lo(2 * NW - 1, u) for u in range(4)])
            else:
                wait_ring(vbuf, lsem, t - 1)
            l, acc = accumulate(t - 1, p, alpha, l, acc)
            s = _dot_nt(q_scr[g].astype(BF16), kbuf[t & (RING - 1)].reshape(4 * 128, DH))
            s = own_rows([s[:, 128 * u:128 * (u + 1)] for u in range(4)]) * DH ** -0.5
            _start(hi(n, 0), lo(n, 0))
            _start(hi(n, 1), lo(n, 1))

            def softmax():
                _start(hi(n, 2), lo(n, 2))
                m_old = jnp.where(c == 0, -jnp.inf, m)
                m_new = jnp.maximum(m_old, jnp.max(s, axis=1, keepdims=True))
                return m_new, jnp.exp(s - m_new), jnp.exp(m_old - m_new)

            def softmax_and_finish_previous_group():
                o_scr[0], o_scr[1] = normalize(l, acc)
                return softmax()

            def softmax_and_project_previous_group():
                out = softmax()
                is_b, tile, half = 1 - ((g - 1) >> 2), (c - 1) >> 1, (c - 1) & 1
                rows = _ds(512 * is_b + 128 * tile, 128)
                cols = _ds(1024 * ((g - 1) & 3) + 512 * half, 512)
                y_scr[5 * is_b + tile] += _dot_nt(o_scr[half], wo[rows, cols])
                return out

            kind = jnp.where(jnp.logical_or(g == 0, c > 10), 0, jnp.where(c == 0, 1, 2))
            m, p, alpha = lax.switch(kind, [
                softmax, softmax_and_finish_previous_group, softmax_and_project_previous_group])
            _start(hi(n, 3), lo(n, 3))
            return m, p, alpha, l, acc
        return body

    carry = lax.fori_loop(0, 1, attn_step(bk_hi, bv_lo, first=True), (zero,) * 5)
    carry = lax.fori_loop(1, NB - AHEAD, attn_step(bk_hi, bv_lo), carry)
    carry = lax.fori_loop(NB - AHEAD, NT - AHEAD, attn_step(ak_hi, av_lo), carry)
    o_ref[0, :, D_MODEL:640] = y_scr[5, 0:1, 64:128].astype(BF16)
    for j in range(1, 5):
        o_ref[0, :, 512 + 128 * j:640 + 128 * j] = y_scr[5 + j, 0:1].astype(BF16)
    _, p, alpha, l, acc = lax.fori_loop(NT - AHEAD, NT, attn_step(last_hi, last_lo), carry)

    final = last_copy(512, D_MODEL - 512, lsem.at[AHEAD])
    _start([], [final])
    wait_ring(vbuf, lsem, NT - 1)
    o = jnp.concatenate(normalize(*accumulate(NT - 1, p, alpha, l, acc)), axis=1)

    def landed(stream, tile):
        _wait(*[stream(NT + 2 * tile + j, u) for j in range(2) for u in range(4)])

    def project(tile, width=128):
        lanes = pl.ds(128 * tile, width)
        y = _dot_nt(o, wo[lanes, LAST:HID])
        o_ref[0, :, lanes] = (y[0:1] + y_scr[tile, 0:1, 0:width]).astype(BF16)

    landed(last_hi, 0)
    project(0)
    landed(last_hi, 1)
    landed(last_lo, 0)
    project(1)
    project(2)
    landed(last_lo, 1)
    project(3)
    final.wait()
    project(4, D_MODEL - 512)


@jax.jit
def pallas_concat_heads__gqa_block_cached__sliding_block_cached__decode_kernel(
    A_x: jax.Array,
    A_k_cache: jax.Array,
    A_v_cache: jax.Array,
    A_wq: jax.Array,
    A_wo: jax.Array,
    B_x: jax.Array,
    B_k_cache: jax.Array,
    B_v_cache: jax.Array,
    B_wq: jax.Array,
    B_wo: jax.Array,
):
    for x, k, v, wq, wo in ((A_x, A_k_cache, A_v_cache, A_wq, A_wo),
                            (B_x, B_k_cache, B_v_cache, B_wq, B_wo)):
        assert x.shape == (1, 1, D_MODEL) and k.shape == v.shape == (1, HKV, SK, DH)
        assert wq.shape == (D_MODEL, HID) and wo.shape == (HID, D_MODEL)

    a_shape, b_shape = (HKV, 2, SK // 2, DH), (HKV, SK, DH)
    return pl.pallas_call(
        _kernel,
        in_specs=[pl.BlockSpec(memory_space=pltpu.HBM)] * 10,
        out_shape=jax.ShapeDtypeStruct((1, 1, 2 * D_MODEL), BF16),
        scratch_shapes=[
            pltpu.VMEM((2, 1, D_MODEL), BF16),
            pltpu.VMEM((2, D_MODEL, HID), BF16),
            pltpu.VMEM((2 * D_MODEL, HID), BF16),
            pltpu.VMEM((RING, 4, 2, 64, DH), BF16),
            pltpu.VMEM((RING, 4, 2, 64, DH), BF16),
            pltpu.VMEM((8, 8, DH), F32),
            pltpu.VMEM((2, 8, 4 * DH), BF16),
            pltpu.VMEM((10, 8, 128), F32),
            pltpu.SemaphoreType.DMA(()),
            pltpu.SemaphoreType.DMA((RING,)),
            pltpu.SemaphoreType.DMA((RING,)),
        ],
        compiler_params=pltpu.CompilerParams(
            vmem_limit_bytes=48 * 2**20,
            disable_bounds_checks=True,
            disable_semaphore_checks=True,
        ),
    )(A_x, A_k_cache.reshape(a_shape), A_v_cache.reshape(a_shape), A_wq, A_wo.T,
      B_x, B_k_cache.reshape(b_shape), B_v_cache.reshape(b_shape), B_wq, B_wo.T)
```
